```python
import os as _os
_os.environ.setdefault('JAX_PLATFORMS', 'cpu')
import jax
import jax.numpy as jnp

def _softmax(x, axis=-1):
    return jax.nn.softmax(x, axis=axis)

def _gelu(x):
    return jax.nn.gelu(x, approximate=True)

def _silu(x):
    return jax.nn.silu(x)

def _sigmoid(x):
    return jax.nn.sigmoid(x)

def _layernorm(x, axis=-1, eps=1e-05):
    m = jnp.mean(x, axis=axis, keepdims=True)
    v = jnp.var(x, axis=axis, keepdims=True)
    return (x - m) / jnp.sqrt(v + eps)

def _scatter_add(tgt, idx, src, axis=0):
    return tgt.at[idx].add(src)

def _segment_sum(src, seg, n):
    return jax.ops.segment_sum(src, seg, n)

class _Rng:

    def __init__(self, key):
        self._k = key

    def _next(self):
        self._k, sub = jax.random.split(self._k)
        return sub

    def normal(self, shape):
        return jax.random.normal(self._next(), shape, dtype=jnp.bfloat16)

    def randint(self, lo, hi, shape):
        return jax.random.randint(self._next(), shape, lo, hi, dtype=jnp.int32)

    def uniform(self, shape, lo=0.0, hi=1.0):
        return jax.random.uniform(self._next(), shape, jnp.bfloat16, lo, hi)

    def permutation(self, n):
        return jax.random.permutation(self._next(), n)
kernel_name = 'standalone__conformer_conv_module__speech'

def setup_inputs():
    _rng = _Rng(jax.random.key(int.from_bytes(__import__("os").urandom(4), "little")))
    _w = lambda a: (lambda t: t.astype(jnp.bfloat16) if jnp.issubdtype(t.dtype, jnp.floating) else t)(jnp.asarray(a))
    B, T, D, K = (2, 4000, 512, 15)
    return {'x': _w((lambda *s: _rng.normal(s) * 0.2)(B, T, D)), 'w_pw1': _w((lambda *s: _rng.normal(s) * 0.2)(D, 2 * D)), 'dw': _w((lambda *s: _rng.normal(s) * 0.05)(K, D)), 'w_pw2': _w((lambda *s: _rng.normal(s) * 0.05)(D, D))}

def reference(x, w_pw1, dw, w_pw2):
    B, T, D = x.shape
    K = dw.shape[0]
    h = x @ w_pw1
    a, b = (h[..., :D].copy(), h[..., D:].copy())
    h = a * _sigmoid(b)
    pad = K // 2
    hp = jnp.pad(h, ((0, 0), (pad, pad), (0, 0)))
    out = jnp.zeros_like(h)
    for i in range(K):
        out = out + hp[:, i:i + T, :] * dw[i][None, None, :]
    return _silu(out) @ w_pw2
```

```python
import jax
import jax.numpy as jnp
import jax.experimental.pallas as pl
import jax.experimental.pallas.tpu as pltpu
from jax import lax

F32 = jnp.float32
BF16 = jnp.bfloat16
U32 = jnp.uint32

def make(M=400, UN=2, PRO=2, flags=None, NS=4, lastsplit=True, semchk=True, ppos=(0, 1, 3, 3), ppos_mid=None, NDW=1, dyn_dw=True, npull=3):
    ppos_mid = ppos_mid or ppos
    def kernel(x, w_pw1, dw, w_pw2):
        B, T, D = x.shape
        K = dw.shape[0]
        NC = T // M
        N = B * NC
        NL = D // 128
        R = B * T
        HB = 24
        x2 = x.reshape(R, D)

        def body(x_hbm, w1_hbm, dw_hbm, w2_hbm, o_hbm,
                 xb, ob, w1b, w2b, dwb, dwf, zs, wsem, osem, *bufs):
            hbufs = bufs[:NL * UN]
            hs = [hbufs[u * NL:(u + 1) * NL] for u in range(UN)]
            ss = bufs[NL * UN:]

            def aligned(v, m):
                return v if isinstance(v, int) else pl.multiple_of(v, m)

            def xcopy(c):
                r = pl.ds(aligned(c * M, 16), M)
                return pltpu.make_async_copy(x_hbm.at[r], xb.at[r], wsem.at[2 * NL + 2 + c % NS])

            def ocopy(c):
                if isinstance(c, int) and c == 0:
                    return pltpu.make_async_copy(ob.at[pl.ds(8, M - 8)], o_hbm.at[pl.ds(0, M - 8)], osem.at[0])
                return pltpu.make_async_copy(ob.at[pl.ds(aligned(c * M, 16), M)],
                                             o_hbm.at[pl.ds(aligned(c * M - 8, 8), M)], osem.at[0])

            def w1copy(t):
                return pltpu.make_async_copy(w1_hbm.at[:, pl.ds(t * 128, 128)], w1b.at[t], wsem.at[t])

            w2copy = [pltpu.make_async_copy(w2_hbm.at[:, pl.ds(t * 128, 128)], w2b.at[t], wsem.at[2 * NL]) for t in range(NL)]
            dwcopy = pltpu.make_async_copy(dw_hbm, dwb, wsem.at[2 * NL + 1])
            zero = jnp.zeros((8, 128), F32)

            def mm1(c, u, j, boundary, first=False, pre_b=None):
                h = hs[u][j]
                xv = xb[pl.ds(aligned(c * M, 16), M), :]
                a = jnp.dot(xv, w1b[j], preferred_element_type=F32)
                if pre_b is not None:
                    pre_b()
                b = jnp.dot(xv, w1b[NL + j], preferred_element_type=F32)
                g = a * (0.5 * jnp.tanh(0.5 * b) + 0.5)
                if first:
                    h[0:8, :] = zero
                    h[8:16, :] = zero
                    h[16:24, :] = zero
                    h[HB:HB + 8, :] = zero
                else:
                    tail = hs[(u - 1) % UN][j][HB + M - 8:HB + M + 8, :]
                    h[0:16, :] = tail
                    h[16:24, :] = jnp.where(boundary, zero, g[0:8])
                    h[HB:HB + 8, :] = jnp.where(boundary, zero, tail[8:16])
                if isinstance(c, int) and c == N - 1:
                    h[HB + M + 8:HB + M + 16, :] = zero
                h[HB + 8:HB + M - 8 * npull, :] = g[0:M - 8 - 8 * npull]
                h[pl.ds(pl.multiple_of(zs[0], 8), 8), :] = g[M - 8:M]
                if npull:
                    h[HB + M - 8 * npull:HB + M, :] = g[M - 8 - 8 * npull:M - 8]

            def conv_tile(h, w, t):
                base = 1 if t == 0 else HB + 8 * t - 7
                acc = None
                for k in range(K):
                    p = h[pl.ds(base + k, 8), :] * w[k]
                    acc = p if acc is None else acc + p
                return acc * (0.5 * jnp.tanh(0.5 * acc) + 0.5)

            def s_store(q, j, v, lo, hi):
                sv = jnp.concatenate([lo, hi], axis=0).astype(BF16)
                r = pl.multiple_of(zs[1], 8) if (j == NL - 1 and v == M // 16 - 1) else 8 * v
                ss[q][j, pl.ds(r, 8), :] = pltpu.bitcast(sv, U32)

            def conv(u, j, last):
                h = hs[u][j]
                z = zs[2 + u] if dyn_dw else u % NDW
                w = [dwf[z, k, :, j * 128:(j + 1) * 128] for k in range(K)]
                if last:
                    s_store(u, j, M // 16, conv_tile(h, w, M // 8), zero)
                for v in range(M // 16):
                    s_store(u, j, v, conv_tile(h, w, 2 * v), conv_tile(h, w, 2 * v + 1))

            def mm2(c, q, t, rows=M):
                sv = jnp.concatenate([pltpu.bitcast(ss[q][j, 0:rows // 2, :], BF16) for j in range(NL)], axis=1)
                o = jnp.dot(sv, w2b[t], preferred_element_type=F32)
                ob[pl.ds(aligned(c * M, 16), rows), t * 128:(t + 1) * 128] = o.astype(BF16)

            def step(c, u, pp, start_x=True):
                static = isinstance(c, int)
                first = static and c == 0
                if start_x and not first:
                    xcopy(c + 2).start()
                xcopy(c).wait()
                for j in range(NL):
                    if first:
                        w1copy(j).wait()
                        if j == 0:
                            xcopy(1).start()
                            for cp in w2copy:
                                cp.start()
                            xcopy(2).start()
                        mm1(c, u, j, False, first=True, pre_b=lambda: w1copy(NL + j).wait())
                        if j == 0:
                            dwcopy.wait()
                            dv = dwb[...].astype(F32)
                            for k in range(K):
                                for z in range(NDW):
                                    dwf[z, k] = jnp.broadcast_to(dv[k:k + 1, :], (8, D))
                    else:
                        mm1(c, u, j, (c % NC) == 0)
                    conv(u, j, static and c == N - 1)
                    if not first:
                        for t in range(NL):
                            if pp[t] == j:
                                if static and c == 1 and t == 0:
                                    for cp in w2copy:
                                        cp.wait()
                                mm2(c - 1, (u - 1) % UN, t)
                if not first:
                    ocopy(c - 1).start()

            xcopy(0).start()
            for j in range(NL):
                w1copy(j).start()
                w1copy(NL + j).start()
                if j == 0:
                    dwcopy.start()
            zs[0] = HB + M
            zs[1] = M // 2 - 8
            for u in range(UN):
                zs[2 + u] = 0
            for c in range(PRO):
                step(c, (c - PRO) % UN, ppos if c == PRO - 1 else ppos_mid)

            nloop = (N - 2 - PRO) // UN
            def lb(it, carry):
                for u in range(UN):
                    step(PRO + it * UN + u, u, ppos if u == UN - 1 else ppos_mid)
                return carry
            lax.fori_loop(0, nloop, lb, 0)
            for c in range(PRO + nloop * UN, N):
                step(c, (c - PRO) % UN, ppos if c == N - 1 else ppos_mid, start_x=(c + 2 < N))

            q = (N - 1 - PRO) % UN
            r0 = (N - 1) * M
            for t in range(NL):
                mm2(N - 1, q, t, rows=M + 16)
                if lastsplit:
                    pltpu.make_async_copy(ob.at[pl.ds(r0, M + 8), pl.ds(t * 128, 128)],
                                          o_hbm.at[pl.ds(r0 - 8, M + 8), pl.ds(t * 128, 128)], osem.at[0]).start()
            if not lastsplit:
                pltpu.make_async_copy(ob.at[pl.ds(r0, M + 8)], o_hbm.at[pl.ds(r0 - 8, M + 8)], osem.at[0]).start()
            pltpu.make_async_copy(ob.at[pl.ds(8, R)], o_hbm, osem.at[0]).wait()

        anyspec = pl.BlockSpec(memory_space=pl.ANY)
        sshape = pltpu.VMEM((NL, M // 2 + 8, 128), U32)
        out = pl.pallas_call(
            body,
            in_specs=[anyspec] * 4,
            out_specs=anyspec,
            out_shape=jax.ShapeDtypeStruct((R, D), x.dtype),
            scratch_shapes=[
                pltpu.VMEM((R, D), BF16),
                pltpu.VMEM((R + 16, D), BF16),
                pltpu.VMEM((2 * NL, D, 128), BF16),
                pltpu.VMEM((NL, D, 128), BF16),
                pltpu.VMEM((K, D), BF16),
                pltpu.VMEM((NDW, K, 8, D), F32),
                pltpu.SMEM((2 + UN,), jnp.int32),
                pltpu.SemaphoreType.DMA((2 * NL + 2 + NS,)),
                pltpu.SemaphoreType.DMA((1,)),
            ] + [pltpu.VMEM((HB + M + 16, 128), F32)] * (NL * UN) + [sshape] * UN,
            compiler_params=pltpu.CompilerParams(vmem_limit_bytes=64 * 1024 * 1024, flags=flags,
                                                 disable_semaphore_checks=not semchk),
            name="conf_v3",
        )(x2, w_pw1, dw, w_pw2)
        return out.reshape(B, T, D)
    return kernel


_kernel = make(**dict(flags={'XLA_TPU_FORCE_LP_LLO_SCHEDULER':True,'XLA_TPU_RESCHEDULE_DMA_DONES':True},UN=4,ppos_mid=(0,1,2,3)))


@jax.jit
def pallas_standalone__conformer_conv_module__speech_kernel(x: jax.Array, w_pw1: jax.Array, dw: jax.Array, w_pw2: jax.Array):
    return _kernel(x, w_pw1, dw, w_pw2)
```

```python
import jax
import jax.numpy as jnp
import jax.experimental.pallas as pl
import jax.experimental.pallas.tpu as pltpu
from jax import lax

_LANES = 128
_HALO = 24
_LAG = 16
_WAIT_AHEAD = 48
_TAIL_ROWS = 112
_NEG_LOG2E = -1.4426950408889634


def _sigmoid(v):
    return pltpu.reciprocal(1.0 + jnp.exp2(v * _NEG_LOG2E), approx=True)


def _chunk_sizes(rows):
    head, tail = (352, 352), (480, 352)
    tiles = (rows - sum(head) - sum(tail)) // 16
    n = pl.cdiv(tiles, 26)
    middle = tuple(16 * (tiles // n + (i < tiles % n)) for i in range(n))
    return head + middle + tail


def _aligned(v, m):
    return v if isinstance(v, int) else pl.multiple_of(v, m)


def _conformer_conv_module(x, w_pw1, dw, w_pw2):
    f32, bf16 = jnp.float32, jnp.bfloat16
    B, T, D = x.shape
    K = dw.shape[0]
    NL = D // _LANES
    assert T % 16 == 0 and T >= 2400 and NL == 4 and D == NL * _LANES
    assert K % 2 == 1 and K // 2 <= 7

    sizes = _chunk_sizes(T)
    NCH = len(sizes)
    last = NCH - 1
    starts = [sum(sizes[:c]) for c in range(NCH + 1)]
    ostarts = [0] + [r - _LAG for r in starts[1:-1]] + [T]
    osizes = [q - p for p, q in zip(ostarts[:-1], ostarts[1:])]
    xcuts = starts[:5] + [T]
    NG = len(xcuts) - 1
    w1_order = [t for j in range(NL) for t in (j, NL + j)]

    def pw2_slots(c):
        if c == 1:
            return (1, 1, 2, 3)
        if c == last:
            return (0, 1, 3, 3)
        return (0, 1, 2, 3)

    def out_pieces(c, t):
        n = osizes[c]
        if c < last - 1:
            return [((0, n), (0, D))] if t == NL - 1 else []
        cols = (t * _LANES, (t + 1) * _LANES)
        if c == last and t == NL - 1:
            return [((0, n - _TAIL_ROWS), cols), ((n - _TAIL_ROWS, n), cols)]
        return [((0, n), cols)]

    def kernel(x_hbm, w1_hbm, dw_hbm, w2_hbm, o_hbm,
               x_buf, w1_buf, w2_buf, dw_buf, taps, offs, out_sem, *bufs):
        o_bufs = bufs[:NCH]
        s_bufs = bufs[NCH:2 * NCH]
        h_bufs = [bufs[2 * NCH + c * NL:2 * NCH + (c + 1) * NL] for c in range(NCH)]

        def out_copy(b, c, rows, cols):
            (p, q), cols = rows, pl.ds(cols[0], cols[1] - cols[0])
            dst = pl.ds(_aligned(b * T + ostarts[c] + p, 16), q - p)
            return pltpu.make_async_copy(
                o_bufs[c].at[b, pl.ds(p, q - p), cols], o_hbm.at[dst, cols], out_sem.at[0])


        def glu(c, j, value, gate):
            h, m = h_bufs[c][j], sizes[c]
            g = value * _sigmoid(gate)
            h[_HALO:_HALO + m - 40, :] = g[:m - 40]
            h[_HALO + m - 16:_HALO + m - 8, :] = g[m - 16:m - 8]
            h[pl.ds(pl.multiple_of(offs[0, c], 8), 8), :] = g[m - 8:]
            h[_HALO + m - 40:_HALO + m - 16, :] = g[m - 40:m - 16]
            if c < last:
                h_bufs[c + 1][j][0:_HALO, :] = g[m - _HALO:]

        def conv_silu(c, j, zero):
            h, n = h_bufs[c][j], osizes[c]
            first = _HALO + ostarts[c] - starts[c] - K // 2
            acc = None
            for k in range(K):
                tap = taps[zero, k, :, j * _LANES:(j + 1) * _LANES]
                term = h[pl.ds(first + k, n), :].reshape(n // 8, 8, _LANES) * tap[None]
                acc = term if acc is None else acc + term
            acc = acc.reshape(n, _LANES)
            s = (acc * _sigmoid(acc)).astype(bf16)
            if j < NL - 1:
                s_bufs[c][j] = s
            else:
                s_bufs[c][j, 0:n - 16, :] = s[:n - 16]
                s_bufs[c][j, pl.ds(pl.multiple_of(offs[1, c], 16), 16), :] = s[n - 16:]

        def pw2_pass(b, c, t):
            s = jnp.concatenate([s_bufs[c][j] for j in range(NL)], axis=1)
            o = jnp.dot(s, w2_buf[t], preferred_element_type=f32).astype(bf16)
            cols = slice(t * _LANES, (t + 1) * _LANES)
            pieces = out_pieces(c, t)
            if len(pieces) > 1:
                for (p, q), span in pieces:
                    o_bufs[c][b, p:q, cols] = o[p:q]
                    out_copy(b, c, (p, q), span).start()
            else:
                o_bufs[c][b, :, cols] = o
                for rows, span in pieces:
                    out_copy(b, c, rows, span).start()

        def compute(in_sems):
            def w1_copy(t):
                return pltpu.make_async_copy(
                    w1_hbm.at[:, pl.ds(t * _LANES, _LANES)], w1_buf.at[t], in_sems.at[t])

            def w2_copy(t):
                return pltpu.make_async_copy(
                    w2_hbm.at[:, pl.ds(t * _LANES, _LANES)], w2_buf.at[t], in_sems.at[2 * NL + t])

            def x_copy(b, g):
                rows = pl.ds(_aligned(b * T + xcuts[g], 16), xcuts[g + 1] - xcuts[g])
                return pltpu.make_async_copy(
                    x_hbm.at[rows], x_buf.at[rows], in_sems.at[3 * NL + 1 + b * NG + g])

            dw_copy = pltpu.make_async_copy(dw_hbm, dw_buf, in_sems.at[3 * NL])

            def batch(b, carry):
                only_first = pl.when(b == 0)
                zero = offs[2, 0]

                def x_rows(lo, hi):
                    return x_buf[pl.ds(_aligned(b * T + lo, 16), hi - lo), :]

                def pw1_while_loading(i):
                    m = sizes[0]
                    early = x_rows(0, m - _WAIT_AHEAD)
                    w = w1_buf[w1_order[i]]
                    if i + 1 < 2 * NL:
                        only_first(lambda: w1_copy(w1_order[i + 1]).wait())
                    else:
                        x_copy(b, 1).wait()
                    xv = jnp.concatenate([early, x_rows(m - _WAIT_AHEAD, m)], axis=0)
                    return jnp.dot(xv, w, preferred_element_type=f32)

                x_copy(b, 0).wait()
                for c in range(NCH):
                    if 1 < c < NG:
                        x_copy(b, c).wait()
                    for j in range(NL):
                        if c == 0:
                            value = pw1_while_loading(2 * j)
                            gate = pw1_while_loading(2 * j + 1)
                        else:
                            xv = x_rows(starts[c], starts[c + 1])
                            value = jnp.dot(xv, w1_buf[j], preferred_element_type=f32)
                            gate = jnp.dot(xv, w1_buf[NL + j], preferred_element_type=f32)
                        glu(c, j, value, gate)
                        for t in range(NL):
                            if c > 0 and pw2_slots(c)[t] == j:
                                if c == 1:
                                    only_first(lambda: w2_copy(t).wait())
                                pw2_pass(b, c - 1, t)
                        conv_silu(c, j, zero)
                for t in range(NL):
                    pw2_pass(b, last, t)
                return carry

            dw_copy.start()
            w1_copy(w1_order[0]).start()
            x_copy(0, 0).start()
            for t in w1_order[1:]:
                w1_copy(t).start()
            x_copy(0, 1).start()
            for t in range(NL):
                w2_copy(t).start()
            for b in range(B):
                for g in range(2 if b == 0 else 0, NG):
                    x_copy(b, g).start()

            for c in range(NCH):
                offs[0, c] = _HALO + sizes[c] - 8
                offs[1, c] = osizes[c] - 16
            offs[2, 0] = 0
            for j in range(NL):
                h_bufs[0][j][_HALO - 8:_HALO, :] = jnp.zeros((8, _LANES), f32)
                h_bufs[last][j][_HALO + sizes[last]:, :] = jnp.zeros((8, _LANES), f32)
            dw_copy.wait()
            dw_f32 = dw_buf[...].astype(f32)
            for k in range(K):
                taps[0, k] = jnp.broadcast_to(dw_f32[k:k + 1, :], (8, D))
            w1_copy(w1_order[0]).wait()
            lax.fori_loop(0, B, batch, 0)

        pl.run_scoped(compute, pltpu.SemaphoreType.DMA((3 * NL + 1 + B * NG,)))
        for b in range(B):
            for c in range(NCH):
                for t in range(NL):
                    for rows, span in out_pieces(c, t):
                        out_copy(b, c, rows, span).wait()

    hbm = pl.BlockSpec(memory_space=pl.ANY)
    out = pl.pallas_call(
        kernel,
        in_specs=[hbm] * 4,
        out_specs=hbm,
        out_shape=jax.ShapeDtypeStruct((B * T, D), x.dtype),
        scratch_shapes=[
            pltpu.VMEM((B * T, D), bf16),
            pltpu.VMEM((2 * NL, D, _LANES), bf16),
            pltpu.VMEM((NL, D, _LANES), bf16),
            pltpu.VMEM((K, D), bf16),
            pltpu.VMEM((1, K, 8, D), f32),
            pltpu.SMEM((3, NCH), jnp.int32),
            pltpu.SemaphoreType.DMA((1,)),
        ]
        + [pltpu.VMEM((B, n, D), bf16) for n in osizes]
        + [pltpu.VMEM((NL, n, _LANES), bf16) for n in osizes]
        + [pltpu.VMEM((_HALO + m + 8, _LANES), f32) for m in sizes for _ in range(NL)],
        compiler_params=pltpu.CompilerParams(
            vmem_limit_bytes=64 * 1024 * 1024,
            disable_bounds_checks=True,
            flags={
                "XLA_TPU_FORCE_LP_LLO_SCHEDULER": True,
                "XLA_TPU_RESCHEDULE_DMA_DONES": True,
            },
        ),
        name="conformer_conv_module",
    )(x.reshape(B * T, D), w_pw1, dw, w_pw2)
    return out.reshape(B, T, D)


@jax.jit
def pallas_standalone__conformer_conv_module__speech_kernel(
    x: jax.Array,
    w_pw1: jax.Array,
    dw: jax.Array,
    w_pw2: jax.Array,
):
    return _conformer_conv_module(x, w_pw1, dw, w_pw2)
```
